```python
import jax
import jax.numpy as jnp

def _softmax(x, axis=-1):
    return jax.nn.softmax(x, axis=axis)

def _gelu(x):
    return jax.nn.gelu(x, approximate=True)

def _silu(x):
    return jax.nn.silu(x)

def _sigmoid(x):
    return jax.nn.sigmoid(x)

def _layernorm(x, axis=-1, eps=1e-05):
    m = jnp.mean(x, axis=axis, keepdims=True)
    v = jnp.var(x, axis=axis, keepdims=True)
    return (x - m) / jnp.sqrt(v + eps)

def _scatter_add(tgt, idx, src, axis=0):
    return tgt.at[idx].add(src)

def _segment_sum(src, seg, n):
    return jax.ops.segment_sum(src, seg, n)

class _Rng:

    def __init__(self, key):
        self._k = key

    def _next(self):
        self._k, sub = jax.random.split(self._k)
        return sub

    def normal(self, shape):
        return jax.random.normal(self._next(), shape, dtype=jnp.bfloat16)

    def randint(self, lo, hi, shape):
        return jax.random.randint(self._next(), shape, lo, hi, dtype=jnp.int32)

    def uniform(self, shape, lo=0.0, hi=1.0):
        return jax.random.uniform(self._next(), shape, jnp.bfloat16, lo, hi)

    def permutation(self, n):
        return jax.random.permutation(self._next(), n)
kernel_name = 'adaLN_cond__grouped_kv_mqa__dense_activation_silu__prompt'

def _fwd_setup_inputs():
    _rng = _Rng(jax.random.key(int.from_bytes(__import__("os").urandom(4), "little")))
    _w = lambda a: (lambda t: t.astype(jnp.bfloat16) if jnp.issubdtype(t.dtype, jnp.floating) else t)(jnp.asarray(a))

    def _A_setup():
        B, S, D, H = (1, 2048, 640, 32)
        Dh = D // H
        return {'x': _w((lambda *s: _rng.normal(s) * 0.05)(B, S, D)), 'wq': _w((lambda *s: _rng.normal(s) * 0.05)(D, H * Dh)), 'wk': _w((lambda *s: _rng.normal(s) * 0.05)(D, Dh)), 'wv': _w((lambda *s: _rng.normal(s) * 0.05)(D, Dh)), 'wo': _w((lambda *s: _rng.normal(s) * 0.05)(H * Dh, D))}
    _A_in = _A_setup()

    def _B_setup():
        B, S, D, F = (1, 2048, 640, 1728)
        return {'x': _w((lambda *s: _rng.normal(s) * 0.05)(B, S, D)), 'w1': _w((lambda *s: _rng.normal(s) * 0.05)(D, F) * D ** (-0.5)), 'w2': _w((lambda *s: _rng.normal(s) * 0.05)(F, D) * F ** (-0.5))}
    _B_in = _B_setup()
    return {'A_x': _A_in['x'], 'A_wq': _A_in['wq'], 'A_wk': _A_in['wk'], 'A_wv': _A_in['wv'], 'A_wo': _A_in['wo'], 'B_x': _B_in['x'], 'B_w1': _B_in['w1'], 'B_w2': _B_in['w2'], 'c': _w((lambda *s: _rng.normal(s) * 0.05)(1, 640)), 'w_mod': _w((lambda *s: _rng.normal(s) * 0.05)(640, 6 * 640) * 640 ** (-0.5))}

def _fwd_reference(A_x, A_wq, A_wk, A_wv, A_wo, B_x, B_w1, B_w2, c, w_mod):

    def _A_ref(x, wq, wk, wv, wo):
        B, S, D = x.shape
        H = 32
        Dh = D // H
        q = (lambda x, *d: x.transpose(*d))((x @ wq).reshape(B, S, H, Dh), 0, 2, 1, 3)
        k = x @ wk
        v = x @ wv
        scores = jnp.einsum('bhqd,bkd->bhqk', q, k) * Dh ** (-0.5)
        p = _softmax(scores, axis=-1)
        o = jnp.einsum('bhqk,bkd->bhqd', p, v)
        return (lambda x, *d: x.transpose(*d))(o, 0, 2, 1, 3).reshape(B, S, H * Dh) @ wo

    def _B_ref(x, w1, w2):
        h = jnp.einsum('bsd,df->bsf', x, w1)
        h = _silu(h)
        out = jnp.einsum('bsf,fd->bsd', h, w2)
        return out
    x = A_x
    mod = (_silu(c) @ w_mod).reshape(c.shape[0], 6, 1, -1)
    sa, ca, ga, sb, cb, gb = (mod[:, 0].copy(), mod[:, 1].copy(), mod[:, 2].copy(), mod[:, 3].copy(), mod[:, 4].copy(), mod[:, 5].copy())
    h = _layernorm(x, axis=-1) * (1 + ca) + sa
    x = x + ga * _A_ref(h, A_wq, A_wk, A_wv, A_wo)
    h = _layernorm(x, axis=-1) * (1 + cb) + sb
    x = x + gb * _B_ref(h, B_w1, B_w2)
    return x

def setup_inputs():
    _inp = _fwd_setup_inputs()
    _gk = jax.random.fold_in(jax.random.key(int.from_bytes(__import__("os").urandom(4), "little")), 2 ** 31 - 1)
    _shapes = [[1, 2048, 640]]
    _dtypes = ['bfloat16']
    _gks = jax.random.split(_gk, len(_shapes))
    _gs = [jax.random.normal(k, s, dtype=jnp.dtype(d)) * 0.05 for k, s, d in zip(_gks, _shapes, _dtypes)]
    _inp['grad_out'] = _gs[0]
    return _inp

def reference(A_x, A_wq, A_wk, A_wv, A_wo, B_w1, B_w2, c, w_mod, B_x, grad_out):
    _const = dict(B_x=B_x)

    def _f(*_d):
        return _fwd_reference(**{'A_x': _d[0], 'A_wq': _d[1], 'A_wk': _d[2], 'A_wv': _d[3], 'A_wo': _d[4], 'B_w1': _d[5], 'B_w2': _d[6], 'c': _d[7], 'w_mod': _d[8], **_const})
    _out, _vjp = jax.vjp(_f, A_x, A_wq, A_wk, A_wv, A_wo, B_w1, B_w2, c, w_mod)
    _grads = _vjp(grad_out)
    _out0 = jnp.asarray(_out)
    return (_out0, *[jnp.asarray(_g) for _g in _grads])
```

```python
import math

import jax
import jax.numpy as jnp
from jax import lax
import jax.experimental.pallas as pl
import jax.experimental.pallas.tpu as pltpu

S = 2048
D = 640
H = 32
DH = 20
F = 1728
TQ = 256
NQ = S // TQ
CK = 128
NC = S // CK
LAG = 4
SL = 32
OFF_B = 12
NF = 2
FC = F // NF
EPS = 1e-5
SCALE = DH ** -0.5
LOG2E = math.log2(math.e)

bf16 = jnp.bfloat16
f32 = jnp.float32
NT = (((1,), (1,)), ((), ()))


def _dot(a, b):
    return jnp.dot(a, b, preferred_element_type=f32)


def _dot_nt(a, b):
    return lax.dot_general(a, b, NT, preferred_element_type=f32)


def _eye(n):
    r = lax.broadcasted_iota(jnp.int32, (n, n), 0)
    c = lax.broadcasted_iota(jnp.int32, (n, n), 1)
    return jnp.where(r == c, 1.0, 0.0).astype(bf16)


def _sigmoid(x):
    return 1.0 / (1.0 + jnp.exp(-x))


def _fold(v):
    r = v[:, 0:128]
    for t in range(1, v.shape[1] // 128):
        r = r + v[:, t * 128:(t + 1) * 128]
    return r


def _kernel(
    x_hbm, wq_hbm, wkT_ref, wvT_ref, wo_hbm, w1T_hbm, w2_hbm, c_ref, wmod_hbm, dy_ref,
    out_ref, dx_hbm, dwq_hbm, dwkT_ref, dwvT_ref, dwo_hbm, dw1T_hbm, dw2_hbm, dc_ref, dwmod_hbm,
    p_scr, s_scr, q_scr, o_scr, do_scr, dq_scr, linv_scr, f_scr, dh2_scr,
    wqT, woT, w1c, w2Tc, modb, xT, h1T, mu1, rs1, dx1T, dh1T,
    kx, vx, kT, vT, dkT, dvT,
    dwq_acc, dwo_acc, dw1T_acc, dw2_acc, dmod_acc, wkvT, dkv_scr, dwkv_acc, dmod_row, scb_scr,
    x_ref, wq_ref, wo_ref, w1T, w2_ref, wmod_ref,
    dwq_ref, dwo_ref, dw1T_ref, dw2_ref, dwmod_ref,
    in_sem, out_sem, dx_sem,
):
    i = pl.program_id(0)
    eye = _eye(128)
    dx_ref = x_ref

    in_pairs = [(x_hbm, x_ref), (wmod_hbm, wmod_ref), (wq_hbm, wq_ref), (wo_hbm, wo_ref),
                (w1T_hbm, w1T), (w2_hbm, w2_ref)]
    in_copies = [pltpu.make_async_copy(s, d, in_sem.at[n]) for n, (s, d) in enumerate(in_pairs)]
    out_pairs = [(dw1T_ref, dw1T_hbm), (dw2_ref, dw2_hbm), (dwo_ref, dwo_hbm), (dwq_ref, dwq_hbm),
                 (dwmod_ref.at[:, 2 * D:], dwmod_hbm.at[:, 2 * D:]),
                 (dwmod_ref.at[:, :2 * D], dwmod_hbm.at[:, :2 * D])]
    out_copies = [pltpu.make_async_copy(s, d, out_sem.at[n]) for n, (s, d) in enumerate(out_pairs)]

    def dx_copy(t):
        rows = pl.ds(pl.multiple_of(t * TQ, TQ), TQ)
        return pltpu.make_async_copy(dx_ref.at[rows, :], dx_hbm.at[rows, :], dx_sem.at[t])

    def cast_into(dst, src, n):
        rows = src.shape[0] // n

        def body(b, carry):
            sl = pl.ds(pl.multiple_of(b * rows, 16), rows)
            dst[sl, :] = src[sl, :].astype(dst.dtype)
            return carry
        lax.fori_loop(0, n, body, 0)

    def dwmod_chunks(lo, hi):
        def body(j, carry):
            dm = jnp.sum(dmod_acc[j].T, axis=0, keepdims=True)
            dmod_row[j] = dm
            c0 = j * D
            for cb in range(0, D, 128):
                dwmod_ref[:, pl.ds(pl.multiple_of(c0 + cb, 128), 128)] = (
                    scb_scr[...] * dm[:, cb:cb + 128]).astype(bf16)
            return carry
        lax.fori_loop(lo, hi, body, 0)

    @pl.when(i == 0)
    def _prologue():
        in_copies[0].start()
        in_copies[1].start()

        def zero(ref, n):
            rows = ref.shape[0] // n

            def body(b, carry):
                ref[pl.ds(b * rows, rows)] = jnp.zeros((rows,) + ref.shape[1:], ref.dtype)
                return carry
            lax.fori_loop(0, n, body, 0)

        def zero2(ref, n):
            rows = ref.shape[0] // n

            def body(b, carry):
                ref[pl.ds(pl.multiple_of(b * rows, 8), rows), :] = jnp.zeros(
                    (rows, ref.shape[1]), ref.dtype)
                return carry
            lax.fori_loop(0, n, body, 0)

        zero(dkT, 2)
        zero(dvT, 2)
        zero(dmod_acc, 6)
        zero2(dwq_acc, 5)
        zero2(dwo_acc, 5)
        zero2(dw1T_acc, 12)
        zero2(dw2_acc, 12)

        r = lax.broadcasted_iota(jnp.int32, (4 * SL, DH), 0)
        cc = lax.broadcasted_iota(jnp.int32, (4 * SL, DH), 1)
        selk = jnp.where((r == cc) | (r == cc + SL + OFF_B), 1.0, 0.0).astype(bf16)
        selv = jnp.where((r == cc + 2 * SL) | (r == cc + 3 * SL + OFF_B), 1.0, 0.0).astype(bf16)
        wkvT[...] = (_dot(selk, wkT_ref[...]) + _dot(selv, wvT_ref[...])).astype(bf16)

        cf = c_ref[...].astype(f32)
        sc = cf * _sigmoid(cf)
        scb_scr[...] = jnp.broadcast_to(sc, (128, D)).T

        in_copies[0].wait()

        def xt_body(t, carry):
            tok = pl.ds(pl.multiple_of(t * TQ, TQ), TQ)
            xt = jnp.concatenate(
                [_dot_nt(eye, x_ref[tok, cb:cb + 128]) for cb in range(0, D, 128)], axis=0)
            xT[:, tok] = xt.astype(bf16)
            mu = jnp.mean(xt, axis=0, keepdims=True)
            xc = xt - mu
            var = jnp.mean(xc * xc, axis=0, keepdims=True)
            mu1[:, tok] = mu
            rs1[:, tok] = lax.rsqrt(var + EPS)
            return carry

        lax.fori_loop(0, NQ, xt_body, 0)

        in_copies[1].wait()
        for n in range(2, 6):
            in_copies[n].start()
        sc16 = jnp.broadcast_to(sc, (16, D)).astype(bf16)
        mod = _dot(sc16, wmod_ref[...])
        for j in range(6):
            row = mod[0:1, j * D:(j + 1) * D]
            if j in (1, 4):
                row = row + 1.0
            colb = jnp.broadcast_to(row, (128, D)).T
            for t in range(TQ // 128):
                modb[j, :, t * 128:(t + 1) * 128] = colb

        rr = lax.broadcasted_iota(jnp.int32, (SL, TQ), 0)

        def tok_body(t, carry):
            t0 = pl.multiple_of(t * TQ, TQ)
            tok = pl.ds(t0, TQ)
            xh = (xT[:, tok].astype(f32) - mu1[:, tok]) * rs1[:, tok]
            h1 = (xh * modb[1] + modb[0]).astype(bf16)
            h1T[:, tok] = h1
            kv = _dot(wkvT[...], h1)
            kvb = kv.astype(bf16)
            kT[0, :, tok] = kvb[0:SL]
            kT[1, :, tok] = kvb[SL:2 * SL]
            vT[0, :, tok] = jnp.where(rr == DH, 1.0, kv[2 * SL:3 * SL]).astype(bf16)
            vT[1, :, tok] = jnp.where(rr == 0, 1.0, kv[3 * SL:4 * SL]).astype(bf16)
            for tb in range(TQ // 128):
                rows = pl.ds(pl.multiple_of(t0 + tb * 128, 128), 128)
                cols = slice(tb * 128, (tb + 1) * 128)
                kx[0, rows, :] = _dot_nt(eye, kvb[0:SL, cols]).astype(bf16)
                kx[1, rows, :] = _dot_nt(eye, kvb[SL:2 * SL, cols]).astype(bf16)
                vx[0, rows, :] = _dot_nt(eye, kvb[2 * SL:3 * SL, cols]).astype(bf16)
                vx[1, rows, :] = _dot_nt(eye, kvb[3 * SL:4 * SL, cols]).astype(bf16)
            return carry

        lax.fori_loop(0, NQ, tok_body, 0)

        in_copies[2].wait()
        in_copies[3].wait()

        def tr_small(b, carry):
            cb = pl.multiple_of(b * 128, 128)
            wqT[pl.ds(cb, 128), :] = _dot_nt(eye, wq_ref[:, pl.ds(cb, 128)]).astype(bf16)
            woT[pl.ds(cb, 128), :] = _dot_nt(eye, wo_ref[:, pl.ds(cb, 128)]).astype(bf16)
            return carry
        lax.fori_loop(0, D // 128, tr_small, 0)

        in_copies[4].wait()
        in_copies[5].wait()

        def tr_big(b, carry):
            cb = pl.multiple_of(b * 128, 128)
            for c in range(NF):
                rows = slice(c * FC, (c + 1) * FC)
                w1c[c, pl.ds(cb, 128), :] = _dot_nt(eye, w1T[rows, pl.ds(cb, 128)]).astype(bf16)
                w2Tc[c, pl.ds(cb, 128), :] = _dot_nt(
                    eye, w2_ref[rows, pl.ds(cb, 128)]).astype(bf16)
            return carry
        lax.fori_loop(0, D // 128, tr_big, 0)

    tok0 = pl.multiple_of(i * TQ, TQ)
    tok = pl.ds(tok0, TQ)
    h1t = h1T[:, tok]
    q_scr[...] = _dot(wqT[...], h1t) * (SCALE * LOG2E)

    row24 = lax.broadcasted_iota(jnp.int32, (24, TQ), 0)
    row32 = lax.broadcasted_iota(jnp.int32, (SL, TQ), 0)

    def slab(ref, j, v):
        base = pl.multiple_of(j * 40 + 8 * v, 8)
        return ref[pl.ds(base, SL), :]

    def merge_store(ref, j, a, b):
        base = pl.multiple_of(j * 40, 8)
        ref[pl.ds(base, 8), :] = a[0:8]
        ref[pl.ds(base + 8, 24), :] = jnp.where(row24 < DH - 8, a[8:32], b[0:24])
        ref[pl.ds(base + 32, 8), :] = b[24:32]

    def fwd_step(h_cur, v_cur, qn, v_next, m):
        mx = None
        acc = None
        for c in range(NC):
            sl = pl.ds(c * CK, CK)
            p = jnp.exp2(s_scr[sl, :] - m).astype(bf16)
            s = _dot(kx[v_next, sl, :], qn)
            s_scr[sl, :] = s
            cm = jnp.max(s.reshape(CK // 8, 8, TQ), axis=0)
            mx = cm if mx is None else jnp.maximum(mx, cm)
            p_scr[h_cur, sl, :] = p
            d = _dot(vT[v_cur, :, sl], p)
            acc = d if acc is None else acc + d
        return acc, jnp.max(mx, axis=0, keepdims=True)

    s0 = _dot(kx[0], slab(q_scr, 0, 0).astype(bf16))
    s_scr[...] = s0
    m0 = jnp.max(s0, axis=0, keepdims=True)

    def fwd_body(j, m):
        qb = slab(q_scr, j, 1).astype(bf16)
        oa, m = fwd_step(2 * j, 0, qb, 1, m)
        qn = slab(q_scr, jnp.minimum(j + 1, H // 2 - 1), 0).astype(bf16)
        ob, m = fwd_step(2 * j + 1, 1, qn, 0, m)
        la = 1.0 / oa[DH:DH + 1]
        lb = 1.0 / ob[0:1]
        linv_scr[j, 0:1, :] = la
        linv_scr[j, 1:2, :] = lb
        merge_store(o_scr, j, oa * la, ob * lb)
        return m

    lax.fori_loop(0, H // 2, fwd_body, m0)

    oT = o_scr[...].astype(bf16)
    aT = _dot(woT[...], oT)
    dyT = jnp.concatenate(
        [_dot_nt(eye, dy_ref[:, cb:cb + 128]) for cb in range(0, D, 128)], axis=0)
    df = (dyT * modb[5]).astype(bf16)
    x1 = xT[:, tok].astype(f32) + modb[2] * aT
    mu2 = jnp.mean(x1, axis=0, keepdims=True)
    xc2 = x1 - mu2
    var2 = jnp.mean(xc2 * xc2, axis=0, keepdims=True)
    rs2 = lax.rsqrt(var2 + EPS)
    xh2 = xc2 * rs2
    h2 = (xh2 * modb[4] + modb[3]).astype(bf16)
    f_scr[...] = jnp.zeros_like(f_scr)
    dh2_scr[...] = jnp.zeros_like(dh2_scr)

    def mlp_body(c, carry):
        rows = pl.ds(pl.multiple_of(c * FC, 16), FC)
        u = _dot(w1T[rows, :], h2)
        dg = _dot(w2_ref[rows, :], df)
        sg = _sigmoid(u)
        g = (u * sg).astype(bf16)
        du = (dg * (sg * (1.0 + u * (1.0 - sg)))).astype(bf16)
        f_scr[...] += _dot(w2Tc[c], g)
        dw2_acc[rows, :] += _dot_nt(g, df)
        dh2_scr[...] += _dot(w1c[c], du)
        dw1T_acc[rows, :] += _dot_nt(du, h2)
        return carry

    lax.fori_loop(0, NF, mlp_body, 0)

    fT = f_scr[...]
    dh2 = dh2_scr[...]
    yT = (x1 + modb[5] * fT).astype(bf16)
    for tb in range(TQ // 128):
        out_ref[tb * 128:(tb + 1) * 128, :] = _dot_nt(
            eye, yT[:, tb * 128:(tb + 1) * 128]).astype(bf16)
    dmod_acc[5] += _fold(dyT * fT)
    dmod_acc[3] += _fold(dh2)
    dmod_acc[4] += _fold(dh2 * xh2)
    dxh2 = dh2 * modb[4]
    m1 = jnp.mean(dxh2, axis=0, keepdims=True)
    m2 = jnp.mean(dxh2 * xh2, axis=0, keepdims=True)
    dx1 = dyT + rs2 * (dxh2 - m1 - xh2 * m2)
    dx1T[:, tok] = dx1
    dmod_acc[2] += _fold(dx1 * aT)
    da = (dx1 * modb[2]).astype(bf16)
    do_scr[...] = _dot(wo_ref[...], da)
    dwo_acc[...] += _dot_nt(oT, da)

    @pl.when(i == NQ - 1)
    def _():
        cast_into(dw1T_ref, dw1T_acc, 12)
        cast_into(dw2_ref, dw2_acc, 12)
        cast_into(dwo_ref, dwo_acc, 5)
        for n in range(3):
            out_copies[n].start()
        dwmod_chunks(2, 6)
        out_copies[4].start()

    def bwd_body(j, carry):
        heads = []
        for v in range(2):
            do = slab(do_scr, j, v)
            o = slab(o_scr, j, v)
            valid = (row32 < DH) if v == 0 else (row32 >= OFF_B)
            li = linv_scr[j, v:v + 1, :]
            delta = jnp.sum(jnp.where(valid, do * o, 0.0), axis=0, keepdims=True) * li
            heads.append(dict(h=2 * j + v, v=v, do=(do * li).astype(bf16), delta=delta,
                              q=slab(q_scr, j, v).astype(bf16), acc=None))
        items = [(v, c) for v in range(2) for c in range(NC)]
        dss = {}
        for t in range(len(items) + LAG):
            if t < len(items):
                v, c = items[t]
                hd = heads[v]
                sl = pl.ds(c * CK, CK)
                dp = _dot(vx[v, sl, :], hd['do'])
                p = p_scr[hd['h'], sl, :]
                dss[t] = (p.astype(f32) * (dp - hd['delta'])).astype(bf16)
                dvT[v, :, sl] += _dot_nt(hd['do'], p)
            if t >= LAG:
                v, c = items[t - LAG]
                hd = heads[v]
                sl = pl.ds(c * CK, CK)
                ds = dss.pop(t - LAG)
                d = _dot(kT[v, :, sl], ds)
                hd['acc'] = d if hd['acc'] is None else hd['acc'] + d
                dkT[v, :, sl] += _dot_nt(hd['q'], ds)
        merge_store(dq_scr, j, heads[0]['acc'], heads[1]['acc'])
        return carry

    lax.fori_loop(0, H // 2, bwd_body, 0)

    dq = (dq_scr[...] * SCALE).astype(bf16)
    dwq_acc[...] += _dot_nt(h1t, dq)
    dh1T[:, tok] = _dot(wq_ref[...], dq)

    @pl.when(i == NQ - 1)
    def _epilogue():
        cast_into(dwq_ref, dwq_acc, 5)
        out_copies[3].start()
        rS = lax.broadcasted_iota(jnp.int32, (SL, S), 0)
        dkv_scr[0:SL, :] = jnp.where(rS < DH, dkT[0] * (1.0 / LOG2E), 0.0).astype(bf16)
        dkv_scr[SL:2 * SL, :] = jnp.where(rS >= OFF_B, dkT[1] * (1.0 / LOG2E), 0.0).astype(bf16)
        dkv_scr[2 * SL:3 * SL, :] = jnp.where(rS < DH, dvT[0], 0.0).astype(bf16)
        dkv_scr[3 * SL:4 * SL, :] = jnp.where(rS >= OFF_B, dvT[1], 0.0).astype(bf16)
        wkv = jnp.concatenate(
            [_dot_nt(eye, wkvT[:, cb:cb + 128]) for cb in range(0, D, 128)], axis=0).astype(bf16)
        dwkv_acc[...] = jnp.zeros_like(dwkv_acc)

        def ep_body(t, carry):
            t0 = pl.multiple_of(t * TQ, TQ)
            tk = pl.ds(t0, TQ)
            dkv_t = dkv_scr[:, tk]
            dh1 = dh1T[:, tk] + _dot(wkv, dkv_t)
            dwkv_acc[...] += _dot_nt(dkv_t, h1T[:, tk])
            rs = rs1[:, tk]
            xh1 = (xT[:, tk].astype(f32) - mu1[:, tk]) * rs
            dmod_acc[0] += _fold(dh1)
            dmod_acc[1] += _fold(dh1 * xh1)
            dxh = dh1 * modb[1]
            a1 = jnp.mean(dxh, axis=0, keepdims=True)
            a2 = jnp.mean(dxh * xh1, axis=0, keepdims=True)
            dxt = (dx1T[:, tk] + rs * (dxh - a1 - xh1 * a2)).astype(bf16)
            for tb in range(TQ // 128):
                rows = pl.ds(pl.multiple_of(t0 + tb * 128, 128), 128)
                dx_ref[rows, :] = _dot_nt(eye, dxt[:, tb * 128:(tb + 1) * 128]).astype(bf16)
            dx_copy(t).start()
            return carry

        lax.fori_loop(0, NQ, ep_body, 0)

        dwmod_chunks(0, 2)
        out_copies[5].start()

        dwkv = dwkv_acc[...]
        cc = lax.broadcasted_iota(jnp.int32, (DH, 4 * SL), 0)
        r = lax.broadcasted_iota(jnp.int32, (DH, 4 * SL), 1)
        selk = jnp.where((r == cc) | (r == cc + SL + OFF_B), 1.0, 0.0).astype(bf16)
        selv = jnp.where((r == cc + 2 * SL) | (r == cc + 3 * SL + OFF_B), 1.0, 0.0).astype(bf16)
        hi = dwkv.astype(bf16)
        lo = (dwkv - hi.astype(f32)).astype(bf16)
        dwkT_ref[...] = (_dot(selk, hi) + _dot(selk, lo)).astype(bf16)
        dwvT_ref[...] = (_dot(selv, hi) + _dot(selv, lo)).astype(bf16)

        cf = c_ref[...].astype(f32)
        sgc = _sigmoid(cf)
        dmod = jnp.concatenate([dmod_row[j] for j in range(6)], axis=1)
        dhi = dmod.astype(bf16)
        dlo = (dmod - dhi.astype(f32)).astype(bf16)
        r16 = lax.broadcasted_iota(jnp.int32, (16, 6 * D), 0)
        lhs = jnp.where(r16 == 0, dhi.astype(f32),
                        jnp.where(r16 == 1, dlo.astype(f32), 0.0)).astype(bf16)
        dsc = _dot_nt(lhs, wmod_ref[...])
        dsc = dsc[0:1] + dsc[1:2]
        dc_ref[...] = (dsc * (sgc * (1.0 + cf * (1.0 - sgc)))).astype(bf16)
        for cp in out_copies:
            cp.wait()
        for t in range(NQ):
            dx_copy(t).wait()


@jax.jit
def pallas_adaLN_cond__grouped_kv_mqa__dense_activation_silu__prompt_kernel(
    A_x: jax.Array,
    A_wq: jax.Array,
    A_wk: jax.Array,
    A_wv: jax.Array,
    A_wo: jax.Array,
    B_x: jax.Array,
    B_w1: jax.Array,
    B_w2: jax.Array,
    c: jax.Array,
    w_mod: jax.Array,
    grad_out: jax.Array,
):
    x2 = A_x.reshape(S, D)
    dy2 = grad_out.reshape(S, D)

    def full(shape):
        return pl.BlockSpec(shape, lambda i: (0,) * len(shape))

    hbm = pl.BlockSpec(memory_space=pl.ANY)
    in_specs = [
        hbm, hbm, full((DH, D)), full((DH, D)), hbm, hbm, hbm, full((1, D)), hbm,
        pl.BlockSpec((TQ, D), lambda i: (i, 0)),
    ]
    out_shape = (
        jax.ShapeDtypeStruct((S, D), bf16), jax.ShapeDtypeStruct((S, D), bf16),
        jax.ShapeDtypeStruct((D, D), bf16), jax.ShapeDtypeStruct((DH, D), bf16),
        jax.ShapeDtypeStruct((DH, D), bf16), jax.ShapeDtypeStruct((D, D), bf16),
        jax.ShapeDtypeStruct((F, D), bf16), jax.ShapeDtypeStruct((F, D), bf16),
        jax.ShapeDtypeStruct((1, D), bf16), jax.ShapeDtypeStruct((D, 6 * D), bf16),
    )
    out_specs = (
        pl.BlockSpec((TQ, D), lambda i: (i, 0)),
        hbm, hbm, full((DH, D)), full((DH, D)), hbm, hbm, hbm, full((1, D)), hbm,
    )
    V = pltpu.VMEM
    scratch = [
        V((H, S, TQ), bf16),
        V((S, TQ), f32),
        V((D, TQ), f32),
        V((D, TQ), f32),
        V((D, TQ), f32),
        V((D, TQ), f32),
        V((H // 2, 8, TQ), f32),
        V((D, TQ), f32),
        V((D, TQ), f32),
        V((D, D), bf16), V((D, D), bf16), V((NF, D, FC), bf16), V((NF, D, FC), bf16),
        V((6, D, TQ), f32),
        V((D, S), bf16),
        V((D, S), bf16),
        V((1, S), f32), V((1, S), f32),
        V((D, S), f32), V((D, S), f32),
        V((2, S, SL), bf16), V((2, S, SL), bf16),
        V((2, SL, S), bf16), V((2, SL, S), bf16),
        V((2, SL, S), f32), V((2, SL, S), f32),
        V((D, D), f32), V((D, D), f32), V((F, D), f32), V((F, D), f32),
        V((6, D, 128), f32),
        V((4 * SL, D), bf16),
        V((4 * SL, S), bf16),
        V((4 * SL, D), f32),
        V((6, 1, D), f32),
        V((D, 128), f32),
        V((S, D), bf16), V((D, D), bf16), V((D, D), bf16), V((F, D), bf16), V((F, D), bf16),
        V((D, 6 * D), bf16),
        V((D, D), bf16), V((D, D), bf16), V((F, D), bf16), V((F, D), bf16),
        V((D, 6 * D), bf16),
        pltpu.SemaphoreType.DMA((6,)), pltpu.SemaphoreType.DMA((6,)),
        pltpu.SemaphoreType.DMA((NQ,)),
    ]
    outs = pl.pallas_call(
        _kernel,
        grid=(NQ,),
        in_specs=in_specs,
        out_specs=out_specs,
        out_shape=out_shape,
        scratch_shapes=scratch,
        compiler_params=pltpu.CompilerParams(
            dimension_semantics=("arbitrary",),
            vmem_limit_bytes=124 * 1024 * 1024,
        ),
    )(x2, A_wq, A_wk.T, A_wv.T, A_wo, B_w1.T, B_w2, c, w_mod, dy2)
    out, dx, dwq, dwkT, dwvT, dwo, dw1T, dw2, dc, dwmod = outs
    return (out.reshape(1, S, D), dx.reshape(1, S, D), dwq, dwkT.T, dwvT.T, dwo, dw1T.T, dw2,
            dc, dwmod)
```

```python
import math

import jax
import jax.numpy as jnp
from jax import lax
import jax.experimental.pallas as pl
import jax.experimental.pallas.tpu as pltpu

S = 2048
D = 640
H = 32
DH = 20
F = 1728
TQ = 256
NQ = S // TQ
CK = 128
NC = S // CK
LAG = 4
LAGF = 3
NP = 4
SL = 32
OFF_B = 12
NF = 2
PPAD = 8
FC = F // NF
EPS = 1e-5
SCALE = DH ** -0.5
LOG2E = math.log2(math.e)

bf16 = jnp.bfloat16
f32 = jnp.float32
NT = (((1,), (1,)), ((), ()))


def _dot(a, b):
    return jnp.dot(a, b, preferred_element_type=f32)


def _dot_nt(a, b):
    return lax.dot_general(a, b, NT, preferred_element_type=f32)


def _eye(n):
    r = lax.broadcasted_iota(jnp.int32, (n, n), 0)
    c = lax.broadcasted_iota(jnp.int32, (n, n), 1)
    return jnp.where(r == c, 1.0, 0.0).astype(bf16)


def _sigmoid(x):
    return 1.0 / (1.0 + jnp.exp(-x))


def _fold(v):
    r = v[:, 0:128]
    for t in range(1, v.shape[1] // 128):
        r = r + v[:, t * 128:(t + 1) * 128]
    return r


RB = 128
BLKS = [slice(b, b + RB) for b in range(0, D, RB)]


def _rowsum8(v):
    return jnp.sum(v.reshape(RB // 8, 8, v.shape[1]), axis=0)


def _mean_from(parts):
    return jnp.sum(parts, axis=0, keepdims=True) * (1.0 / D)


def _kernel(
    x_hbm, wq_hbm, wkT_ref, wvT_ref, wo_hbm, w1T_hbm, w2_hbm, c_ref, wmod_hbm, dy_ref,
    out_ref, dx_hbm, dwq_hbm, dwkT_ref, dwvT_ref, dwo_hbm, dw1T_hbm, dw2_hbm, dc_ref, dwmod_hbm,
    p_scr, s_scr, q_all, m_scr, o_scr, do_scr, dq_scr, linv_scr, f_scr, dh2_scr, ds_scr, dqb_scr,
    wqT, woT, w1c, w2Tc, modb, xT, h1T, mu1, rs1, dx1T, dh1T,
    kx, vx, kT, vT, dkT, dvT,
    dwq_acc, dwo_acc, dw1T_acc, dw2_acc, dmod_acc, wkvT, dkv_scr, dwkv_acc, dmod_row, scb_scr,
    x_ref, wq_ref, wo_ref, w1T, w2_ref, wmod_ref,
    dwq_ref, dwo_ref, dw1T_ref, dw2_ref, dwmod_ref,
    in_sem, out_sem, dx_sem, x_sem,
):
    i = pl.program_id(0)
    eye = _eye(128)
    dx_ref = x_ref

    in_pairs = [(wmod_hbm.at[:, :2 * D], wmod_ref.at[:, :2 * D]), (wq_hbm, wq_ref),
                (wmod_hbm.at[:, 2 * D:], wmod_ref.at[:, 2 * D:]), (wo_hbm, wo_ref),
                (w1T_hbm, w1T), (w2_hbm, w2_ref)]
    in_copies = [pltpu.make_async_copy(s, d, in_sem.at[n]) for n, (s, d) in enumerate(in_pairs)]

    def x_copy(t):
        rows = pl.ds(pl.multiple_of(t * TQ, TQ), TQ)
        return pltpu.make_async_copy(x_hbm.at[rows, :], x_ref.at[rows, :], x_sem.at[t])

    out_pairs = [(dw1T_ref, dw1T_hbm), (dw2_ref, dw2_hbm), (dwo_ref, dwo_hbm), (dwq_ref, dwq_hbm),
                 (dwmod_ref.at[:, 2 * D:], dwmod_hbm.at[:, 2 * D:]),
                 (dwmod_ref.at[:, :2 * D], dwmod_hbm.at[:, :2 * D])]
    out_copies = [pltpu.make_async_copy(s, d, out_sem.at[n]) for n, (s, d) in enumerate(out_pairs)]

    def dx_copy(t):
        rows = pl.ds(pl.multiple_of(t * TQ, TQ), TQ)
        return pltpu.make_async_copy(dx_ref.at[rows, :], dx_hbm.at[rows, :], dx_sem.at[t])

    def dwmod_chunks(lo, hi):
        for j in range(lo, hi):
            dm = jnp.sum(dmod_acc[j].T, axis=0, keepdims=True)
            c0 = j * D
            dhi = dm.astype(bf16).astype(f32)
            r16 = lax.broadcasted_iota(jnp.int32, (16, D), 0)
            lhs = jnp.where(r16 == 0, dhi, jnp.where(r16 == 1, dm - dhi, 0.0)).astype(bf16)
            dmod_row[j] = _dot_nt(lhs, wmod_ref[:, c0:c0 + D])
            for cb in range(0, D, 128):
                dwmod_ref[:, c0 + cb:c0 + cb + 128] = (
                    scb_scr[...] * dm[:, cb:cb + 128]).astype(bf16)

    def mod_chunks(sc16, lo, hi):
        for j in range(lo, hi):
            row = _dot(sc16, wmod_ref[:, j * D:(j + 1) * D])[0:1]
            if j in (1, 4):
                row = row + 1.0
            colb = jnp.broadcast_to(row, (128, D)).T
            for t in range(TQ // 128):
                modb[j, :, t * 128:(t + 1) * 128] = colb

    @pl.when(i == 0)
    def _prologue():
        in_copies[0].start()
        x_copy(0).start()
        in_copies[1].start()

        def zero(ref, n):
            rows = ref.shape[0] // n

            def body(b, carry):
                ref[pl.ds(b * rows, rows)] = jnp.zeros((rows,) + ref.shape[1:], ref.dtype)
                return carry
            lax.fori_loop(0, n, body, 0)

        def zero2(ref, n):
            rows = ref.shape[0] // n

            def body(b, carry):
                ref[pl.ds(pl.multiple_of(b * rows, 8), rows), :] = jnp.zeros(
                    (rows, ref.shape[1]), ref.dtype)
                return carry
            lax.fori_loop(0, n, body, 0)

        zero(dkT, 2)
        zero(dvT, 2)
        zero(dmod_acc, 6)
        zero2(s_scr.at[1], 8)
        zero2(o_scr, 2)
        zero2(dq_scr, 2)
        dqb_scr[...] = jnp.zeros_like(dqb_scr)

        r = lax.broadcasted_iota(jnp.int32, (4 * SL, DH), 0)
        cc = lax.broadcasted_iota(jnp.int32, (4 * SL, DH), 1)
        selk = jnp.where((r == cc) | (r == cc + SL + OFF_B), 1.0, 0.0).astype(bf16)
        selv = jnp.where((r == cc + 2 * SL) | (r == cc + 3 * SL + OFF_B), 1.0, 0.0).astype(bf16)
        wkvT[...] = (_dot(selk, wkT_ref[...]) + _dot(selv, wvT_ref[...])).astype(bf16)

        cf = c_ref[...].astype(f32)
        sc = cf * _sigmoid(cf)
        scb_scr[...] = jnp.broadcast_to(sc, (128, D)).T
        sc16 = jnp.broadcast_to(sc, (16, D)).astype(bf16)

        def transpose_sq(dst, src):
            def body(b, carry):
                cb = pl.multiple_of(b * 128, 128)
                dst[pl.ds(cb, 128), :] = _dot_nt(eye, src[:, pl.ds(cb, 128)]).astype(bf16)
                return carry
            lax.fori_loop(0, D // 128, body, 0)

        in_copies[0].wait()
        for t in range(1, NQ):
            x_copy(t).start()
        mod_chunks(sc16, 0, 2)

        rr = lax.broadcasted_iota(jnp.int32, (SL, TQ), 0)

        def stage_a(t):
            tok = pl.ds(pl.multiple_of(t * TQ, TQ), TQ)
            s1 = None
            for bk in BLKS:
                xt = x_ref[tok, bk].astype(f32).T
                xT[bk, tok] = xt.astype(bf16)
                s1 = _rowsum8(xt) if s1 is None else s1 + _rowsum8(xt)
            mu = _mean_from(s1)
            s2 = None
            for bk in BLKS:
                xc = xT[bk, tok].astype(f32) - mu
                s2 = _rowsum8(xc * xc) if s2 is None else s2 + _rowsum8(xc * xc)
            rs = lax.rsqrt(_mean_from(s2) + EPS)
            mu1[:, tok] = mu
            rs1[:, tok] = rs
            for bk in BLKS:
                xh = (xT[bk, tok].astype(f32) - mu) * rs
                h1T[bk, tok] = (xh * modb[1, bk, :] + modb[0, bk, :]).astype(bf16)

        def stage_b(t, h1):
            t0 = pl.multiple_of(t * TQ, TQ)
            tok = pl.ds(t0, TQ)
            kv = _dot(wkvT[...], h1)
            q_all[:, tok] = _dot(wqT[...], h1) * (SCALE * LOG2E)
            kvb = kv.astype(bf16)
            kT[0, :, tok] = kvb[0:SL]
            kT[1, :, tok] = kvb[SL:2 * SL]
            vT[0, :, tok] = jnp.where(rr == DH, 1.0, kv[2 * SL:3 * SL]).astype(bf16)
            vT[1, :, tok] = jnp.where(rr == 0, 1.0, kv[3 * SL:4 * SL]).astype(bf16)
            for tb in range(TQ // 128):
                rows = pl.ds(pl.multiple_of(t0 + tb * 128, 128), 128)
                cols = slice(tb * 128, (tb + 1) * 128)
                kx[0, rows, :] = _dot_nt(eye, kvb[0:SL, cols]).astype(bf16)
                kx[1, rows, :] = _dot_nt(eye, kvb[SL:2 * SL, cols]).astype(bf16)
                vx[0, rows, :] = _dot_nt(eye, kvb[2 * SL:3 * SL, cols]).astype(bf16)
                vx[1, rows, :] = _dot_nt(eye, kvb[3 * SL:4 * SL, cols]).astype(bf16)

        x_copy(0).wait()
        stage_a(0)
        in_copies[1].wait()
        transpose_sq(wqT, wq_ref)

        def tok_body(t, h1):
            x_copy(t + 1).wait()

            @pl.when(t == NQ - 2)
            def _():
                for n in range(2, 6):
                    in_copies[n].start()

            h1c = h1T[:, pl.ds(pl.multiple_of(t * TQ, TQ), TQ)]
            stage_a(t + 1)
            stage_b(t, h1c)
            return h1

        lax.fori_loop(0, NQ - 1, tok_body, 0)
        stage_b(NQ - 1, h1T[:, (NQ - 1) * TQ:NQ * TQ])

        s0 = _dot(kx[0], q_all[0:SL, 0:TQ].astype(bf16))
        s_scr[0] = s0
        m_scr[...] = jnp.max(s0, axis=0, keepdims=True)

    tok0 = pl.multiple_of(i * TQ, TQ)
    tok = pl.ds(tok0, TQ)

    row8 = lax.broadcasted_iota(jnp.int32, (8, TQ), 0)
    row32 = lax.broadcasted_iota(jnp.int32, (SL, TQ), 0)

    def slab(ref, j, v):
        base = pl.multiple_of(j * 40 + 8 * v, 8)
        return ref[pl.ds(base, SL), :]

    def qslab(j, v, tk):
        base = pl.multiple_of(j * 40 + 8 * v, 8)
        return q_all[pl.ds(base, SL), tk].astype(bf16)

    def store_a(ref, j, a):
        ref[pl.ds(pl.multiple_of(j * 40, 8), 24), :] = a[0:24]

    def store_b(ref, j, b):
        mid = pl.ds(pl.multiple_of(j * 40 + 16, 8), 8)
        ref[mid, :] = jnp.where(row8 < 4, ref[mid, :], b[8:16])
        ref[pl.ds(pl.multiple_of(j * 40 + 24, 8), 16), :] = b[16:32]

    def f_produce(v, qn, c, mx):
        sl = pl.ds(c * CK, CK)
        s = _dot(kx[v, sl, :], qn)
        s_scr[v, sl, :] = s
        cm = jnp.max(s.reshape(CK // 8, 8, TQ), axis=0)
        return cm if mx is None else jnp.maximum(mx, cm)

    def f_consume(h, v, c, m, acc):
        sl = pl.ds(c * CK, CK)
        p = jnp.exp2(s_scr[v, sl, :] - m).astype(bf16)
        p_scr[h, pl.ds(c * CK // 2, CK // 2), :] = pltpu.bitcast(p, jnp.uint32)
        d = _dot(vT[v, :, sl], p)
        return d if acc is None else acc + d

    def f_finish(j, v, o):
        if v == 0:
            li = 1.0 / o[DH:DH + 1]
            linv_scr[j, 0:1, :] = li
            store_a(o_scr, j, o * li)
        else:
            li = 1.0 / o[0:1]
            linv_scr[j, 1:2, :] = li
            store_b(o_scr, j, o * li)

    NHI = 2 * NP

    def fwd_body(it, carry):
        m_first, m_bp, acc_bp = carry
        j0 = it * NP
        jp = jnp.maximum(j0 - 1, 0)
        last = it == H // NHI - 1
        qs = [qslab(j0 + (n + 1) // 2, (n + 1) % 2, tok) for n in range(NHI - 1)]
        jn = jnp.where(last, 0, j0 + NP)
        tn0 = pl.multiple_of(jnp.where(last, jnp.minimum(i + 1, NQ - 1), i) * TQ, TQ)
        qs.append(qslab(jn, 0, pl.ds(tn0, TQ)))
        ms = [m_first] + [None] * NHI
        accs = [None] * NHI
        mx = None
        for t in range(NHI * NC):
            n, c = t // NC, t % NC
            mx = f_produce((n + 1) % 2, qs[n], c, mx)
            if c == NC - 1:
                ms[n + 1] = jnp.max(mx, axis=0, keepdims=True)
                mx = None
            u = t - LAGF
            if u < 0:
                acc_bp = f_consume(2 * jp + 1, 1, NC + u, m_bp, acc_bp)
                if u == -1:
                    f_finish(jp, 1, acc_bp)
            else:
                un, uc = u // NC, u % NC
                accs[un] = f_consume(2 * j0 + un, un % 2, uc, ms[un], accs[un])
                if uc == NC - 1:
                    f_finish(j0 + un // 2, un % 2, accs[un])
        return ms[NHI], ms[NHI - 1], accs[NHI - 1]

    m0 = m_scr[...]
    m_next, m_bl, acc_bl = lax.fori_loop(
        0, H // NHI, fwd_body, (m0, m0, jnp.ones((SL, TQ), f32)))
    m_scr[...] = m_next
    for c in range(NC - LAGF, NC):
        acc_bl = f_consume(H - 1, 1, c, m_bl, acc_bl)
    f_finish(H // 2 - 1, 1, acc_bl)

    @pl.when(i == 0)
    def _late_prologue():
        cf = c_ref[...].astype(f32)
        sc16 = jnp.broadcast_to(cf * _sigmoid(cf), (16, D)).astype(bf16)
        in_copies[2].wait()

        mod_chunks(sc16, 2, 6)

        in_copies[3].wait()
        in_copies[4].wait()
        in_copies[5].wait()

        def tr_big(b, carry):
            cb = pl.multiple_of(b * 128, 128)
            woT[pl.ds(cb, 128), :] = _dot_nt(eye, wo_ref[:, pl.ds(cb, 128)]).astype(bf16)
            for c in range(NF):
                rows = slice(c * FC, (c + 1) * FC)
                w1c[c, pl.ds(cb, 128), :] = _dot_nt(eye, w1T[rows, pl.ds(cb, 128)]).astype(bf16)
                w2Tc[c, pl.ds(cb, 128), :] = w2_ref[rows, pl.ds(cb, 128)].astype(f32).T.astype(bf16)
            return carry
        lax.fori_loop(0, D // 128, tr_big, 0)

    first = i == 0

    def accumulate(acc_ref, stage_ref, idx, val):
        new = jnp.where(first, 0.0, acc_ref[idx]) + val
        acc_ref[idx] = new
        stage_ref[idx] = new.astype(bf16)

    tokp = pl.ds(pl.multiple_of(jnp.maximum(i - 1, 0) * TQ, TQ), TQ)
    dyT = dy_ref[...].astype(f32).T
    df = (dyT * modb[5]).astype(bf16)
    oT = o_scr[...].astype(bf16)
    aT = _dot(woT[...], oT)
    dh1T[:, tokp] = _dot(wq_ref[...], dqb_scr[...])
    x1 = xT[:, tok].astype(f32) + modb[2] * aT
    mu2 = jnp.mean(x1, axis=0, keepdims=True)
    xc2 = x1 - mu2
    var2 = jnp.mean(xc2 * xc2, axis=0, keepdims=True)
    rs2 = lax.rsqrt(var2 + EPS)
    xh2 = xc2 * rs2
    h2 = (xh2 * modb[4] + modb[3]).astype(bf16)

    def mlp_body(c, carry):
        rows = pl.ds(pl.multiple_of(c * FC, 16), FC)
        u = _dot(w1T[rows, :], h2)
        dg = _dot(w2_ref[rows, :], df)
        sg = _sigmoid(u)
        g = (u * sg).astype(bf16)
        du = (dg * (sg * (1.0 + u * (1.0 - sg)))).astype(bf16)
        f_scr[...] = jnp.where(c == 0, 0.0, f_scr[...]) + _dot(w2Tc[c], g)
        accumulate(dw2_acc, dw2_ref, (rows, slice(None)), _dot_nt(g, df))
        dh2_scr[...] = jnp.where(c == 0, 0.0, dh2_scr[...]) + _dot(w1c[c], du)
        accumulate(dw1T_acc, dw1T_ref, (rows, slice(None)), _dot_nt(du, h2))
        return carry

    lax.fori_loop(0, NF, mlp_body, 0)

    accumulate(dwq_acc, dwq_ref, (slice(None), slice(None)),
               _dot_nt(h1T[:, tokp], dqb_scr[...]))
    fT = f_scr[...]
    dh2 = dh2_scr[...]
    out_ref[...] = (x1 + modb[5] * fT).T.astype(bf16)
    dmod_acc[5] += _fold(dyT * fT)
    dmod_acc[3] += _fold(dh2)
    dmod_acc[4] += _fold(dh2 * xh2)
    dxh2 = dh2 * modb[4]
    m1 = jnp.mean(dxh2, axis=0, keepdims=True)
    m2 = jnp.mean(dxh2 * xh2, axis=0, keepdims=True)
    dx1 = dyT + rs2 * (dxh2 - m1 - xh2 * m2)
    dx1T[:, tok] = dx1
    dmod_acc[2] += _fold(dx1 * aT)
    da = (dx1 * modb[2]).astype(bf16)
    do_scr[...] = _dot(wo_ref[...], da)
    accumulate(dwo_acc, dwo_ref, (slice(None), slice(None)), _dot_nt(oT, da))

    @pl.when(i == NQ - 1)
    def _():
        for n in range(3):
            out_copies[n].start()
        dwmod_chunks(2, 6)
        out_copies[4].start()

    def b_consume(v, c, ds, q, acc):
        sl = pl.ds(c * CK, CK)
        d = _dot(kT[v, :, sl], ds)
        dkT[v, :, sl] += _dot_nt(q, ds)
        return d if acc is None else acc + d

    ds_scr[...] = jnp.zeros_like(ds_scr)

    def bwd_body(it, acc_bp):
        j0 = it * NP
        jp = jnp.maximum(j0 - 1, 0)
        q_bp = qslab(jp, 1, tok)
        heads = []
        for n in range(NHI):
            j, v = j0 + n // 2, n % 2
            do = slab(do_scr, j, v)
            o = slab(o_scr, j, v)
            valid = (row32 < DH) if v == 0 else (row32 >= OFF_B)
            li = linv_scr[j, v:v + 1, :]
            delta = jnp.sum(jnp.where(valid, do * o, 0.0), axis=0, keepdims=True) * li
            heads.append(dict(h=2 * j + v, do=(do * li).astype(bf16), delta=delta,
                              q=qslab(j, v, tok), acc=None))
        dss = {}
        nt = NHI * NC
        for t in range(nt):
            n, c = t // NC, t % NC
            v = n % 2
            hd = heads[n]
            sl = pl.ds(c * CK, CK)
            u = t - LAG
            if u < 0:
                ds_prev = ds_scr[u + LAG]
            dp = _dot(vx[v, sl, :], hd['do'])
            p = pltpu.bitcast(p_scr[hd['h'], pl.ds(c * CK // 2, CK // 2), :], bf16)
            ds = (p.astype(f32) * (dp - hd['delta'])).astype(bf16)
            if t >= nt - LAG:
                ds_scr[t - (nt - LAG)] = ds
            else:
                dss[t] = ds
            dvT[v, :, sl] += _dot_nt(hd['do'], p)
            if u < 0:
                acc_bp = b_consume(1, NC + u, ds_prev, q_bp, acc_bp)
                if u == -1:
                    store_b(dq_scr, jp, acc_bp)
            else:
                un, uc = u // NC, u % NC
                uh = heads[un]
                uh['acc'] = b_consume(un % 2, uc, dss.pop(u), uh['q'], uh['acc'])
                if uc == NC - 1:
                    (store_a if un % 2 == 0 else store_b)(dq_scr, j0 + un // 2, uh['acc'])
        return heads[NHI - 1]['acc']

    acc_dl = lax.fori_loop(0, H // NHI, bwd_body, jnp.zeros((SL, TQ), f32))
    q_bl = qslab(H // 2 - 1, 1, tok)
    for n in range(LAG):
        acc_dl = b_consume(1, NC - LAG + n, ds_scr[n], q_bl, acc_dl)
    store_b(dq_scr, H // 2 - 1, acc_dl)

    dqb_scr[...] = (dq_scr[...] * SCALE).astype(bf16)

    @pl.when(i == NQ - 1)
    def _epilogue():
        dq = dqb_scr[...]
        dwq_ref[...] = (dwq_acc[...] + _dot_nt(h1T[:, tok], dq)).astype(bf16)
        out_copies[3].start()
        dh1T[:, tok] = _dot(wq_ref[...], dq)
        rS = lax.broadcasted_iota(jnp.int32, (SL, S), 0)
        dkv_scr[0:SL, :] = jnp.where(rS < DH, dkT[0] * (1.0 / LOG2E), 0.0).astype(bf16)
        dkv_scr[SL:2 * SL, :] = jnp.where(rS >= OFF_B, dkT[1] * (1.0 / LOG2E), 0.0).astype(bf16)
        dkv_scr[2 * SL:3 * SL, :] = jnp.where(rS < DH, dvT[0], 0.0).astype(bf16)
        dkv_scr[3 * SL:4 * SL, :] = jnp.where(rS >= OFF_B, dvT[1], 0.0).astype(bf16)
        wkv = jnp.concatenate(
            [_dot_nt(eye, wkvT[:, cb:cb + 128]) for cb in range(0, D, 128)], axis=0).astype(bf16)
        dwkv_acc[...] = jnp.zeros_like(dwkv_acc)

        def ep_tile(t):
            t0 = pl.multiple_of(t * TQ, TQ)
            tk = pl.ds(t0, TQ)
            dkv_t = dkv_scr[:, tk]
            dh1 = dh1T[:, tk] + _dot(wkv, dkv_t)
            dwkv_acc[...] += _dot_nt(dkv_t, h1T[:, tk])
            rs = rs1[:, tk]
            xh1 = (xT[:, tk].astype(f32) - mu1[:, tk]) * rs
            dmod_acc[0] += _fold(dh1)
            dmod_acc[1] += _fold(dh1 * xh1)
            dxh = dh1 * modb[1]
            a1 = jnp.mean(dxh, axis=0, keepdims=True)
            a2 = jnp.mean(dxh * xh1, axis=0, keepdims=True)
            dxt = dx1T[:, tk] + rs * (dxh - a1 - xh1 * a2)
            dx_ref[tk, :] = dxt.T.astype(bf16)

        def ep_body(t2, carry):
            ep_tile(2 * t2)
            ep_tile(2 * t2 + 1)
            dx_copy(2 * t2).start()
            dx_copy(2 * t2 + 1).start()
            return carry

        lax.fori_loop(0, NQ // 2, ep_body, 0)

        dwmod_chunks(0, 2)
        out_copies[5].start()

        dwkv = dwkv_acc[...]
        cc = lax.broadcasted_iota(jnp.int32, (DH, 4 * SL), 0)
        r = lax.broadcasted_iota(jnp.int32, (DH, 4 * SL), 1)
        selk = jnp.where((r == cc) | (r == cc + SL + OFF_B), 1.0, 0.0).astype(bf16)
        selv = jnp.where((r == cc + 2 * SL) | (r == cc + 3 * SL + OFF_B), 1.0, 0.0).astype(bf16)
        hi = dwkv.astype(bf16)
        lo = (dwkv - hi.astype(f32)).astype(bf16)
        dwkT_ref[...] = (_dot(selk, hi) + _dot(selk, lo)).astype(bf16)
        dwvT_ref[...] = (_dot(selv, hi) + _dot(selv, lo)).astype(bf16)

        cf = c_ref[...].astype(f32)
        sgc = _sigmoid(cf)
        dsc = dmod_row[0]
        for j in range(1, 6):
            dsc = dsc + dmod_row[j]
        dsc = dsc[0:1] + dsc[1:2]
        dc_ref[...] = (dsc * (sgc * (1.0 + cf * (1.0 - sgc)))).astype(bf16)
        for cp in out_copies:
            cp.wait()
        for t in range(NQ):
            dx_copy(t).wait()


@jax.jit
def pallas_adaLN_cond__grouped_kv_mqa__dense_activation_silu__prompt_kernel(
    A_x: jax.Array,
    A_wq: jax.Array,
    A_wk: jax.Array,
    A_wv: jax.Array,
    A_wo: jax.Array,
    B_x: jax.Array,
    B_w1: jax.Array,
    B_w2: jax.Array,
    c: jax.Array,
    w_mod: jax.Array,
    grad_out: jax.Array,
):
    x2 = A_x.reshape(S, D)
    dy2 = grad_out.reshape(S, D)

    def full(shape):
        return pl.BlockSpec(shape, lambda i: (0,) * len(shape))

    hbm = pl.BlockSpec(memory_space=pl.ANY)
    in_specs = [
        hbm, hbm, full((DH, D)), full((DH, D)), hbm, hbm, hbm, full((1, D)), hbm,
        pl.BlockSpec((TQ, D), lambda i: (i, 0)),
    ]
    out_shape = (
        jax.ShapeDtypeStruct((S, D), bf16), jax.ShapeDtypeStruct((S, D), bf16),
        jax.ShapeDtypeStruct((D, D), bf16), jax.ShapeDtypeStruct((DH, D), bf16),
        jax.ShapeDtypeStruct((DH, D), bf16), jax.ShapeDtypeStruct((D, D), bf16),
        jax.ShapeDtypeStruct((F, D), bf16), jax.ShapeDtypeStruct((F, D), bf16),
        jax.ShapeDtypeStruct((1, D), bf16), jax.ShapeDtypeStruct((D, 6 * D), bf16),
    )
    out_specs = (
        pl.BlockSpec((TQ, D), lambda i: (i, 0)),
        hbm, hbm, full((DH, D)), full((DH, D)), hbm, hbm, hbm, full((1, D)), hbm,
    )
    V = pltpu.VMEM
    scratch = [
        V((H, S // 2 + PPAD, TQ), jnp.uint32),
        V((2, S, TQ), f32),
        V((D, S), f32),
        V((1, TQ), f32),
        V((D, TQ), f32),
        V((D, TQ), f32),
        V((D, TQ), f32),
        V((H // 2, 8, TQ), f32),
        V((D, TQ), f32),
        V((D, TQ), f32),
        V((LAG, CK, TQ), bf16),
        V((D, TQ), bf16),
        V((D, D), bf16), V((D, D), bf16), V((NF, D, FC), bf16), V((NF, D, FC), bf16),
        V((6, D, TQ), f32),
        V((D, S), bf16),
        V((D, S), bf16),
        V((1, S), f32), V((1, S), f32),
        V((D, S), f32), V((D, S), f32),
        V((2, S, SL), bf16), V((2, S, SL), bf16),
        V((2, SL, S), bf16), V((2, SL, S), bf16),
        V((2, SL, S), f32), V((2, SL, S), f32),
        V((D, D), f32), V((D, D), f32), V((F, D), f32), V((F, D), f32),
        V((6, D, 128), f32),
        V((4 * SL, D), bf16),
        V((4 * SL, S), bf16),
        V((4 * SL, D), f32),
        V((6, 16, D), f32),
        V((D, 128), f32),
        V((S, D), bf16), V((D, D), bf16), V((D, D), bf16), V((F, D), bf16), V((F, D), bf16),
        V((D, 6 * D), bf16),
        V((D, D), bf16), V((D, D), bf16), V((F, D), bf16), V((F, D), bf16),
        V((D, 6 * D), bf16),
        pltpu.SemaphoreType.DMA((6,)), pltpu.SemaphoreType.DMA((6,)),
        pltpu.SemaphoreType.DMA((NQ,)), pltpu.SemaphoreType.DMA((NQ,)),
    ]
    outs = pl.pallas_call(
        _kernel,
        grid=(NQ,),
        in_specs=in_specs,
        out_specs=out_specs,
        out_shape=out_shape,
        scratch_shapes=scratch,
        compiler_params=pltpu.CompilerParams(
            dimension_semantics=("arbitrary",),
            vmem_limit_bytes=124 * 1024 * 1024,
        ),
    )(x2, A_wq, A_wk.T, A_wv.T, A_wo, B_w1.T, B_w2, c, w_mod, dy2)
    out, dx, dwq, dwkT, dwvT, dwo, dw1T, dw2, dc, dwmod = outs
    return (out.reshape(1, S, D), dx.reshape(1, S, D), dwq, dwkT.T, dwvT.T, dwo, dw1T.T, dw2,
            dc, dwmod)
```
